```python
import os as _os
_os.environ.setdefault("JAX_PLATFORMS", "cpu")
import jax
import jax.numpy as jnp

def _softmax(x, axis=-1):
    return jax.nn.softmax(x, axis=axis)
def _gelu(x):
    return jax.nn.gelu(x, approximate=True)
def _silu(x):
    return jax.nn.silu(x)
def _sigmoid(x):
    return jax.nn.sigmoid(x)
def _layernorm(x, axis=-1, eps=1e-5):
    m = jnp.mean(x, axis=axis, keepdims=True)
    v = jnp.var(x, axis=axis, keepdims=True)
    return (x - m) / jnp.sqrt(v + eps)
def _scatter_add(tgt, idx, src, axis=0):
    return tgt.at[idx].add(src)
def _segment_sum(src, seg, n):
    return jax.ops.segment_sum(src, seg, n)
class _Rng:
    def __init__(self, key):
        self._k = key
    def _next(self):
        self._k, sub = jax.random.split(self._k)
        return sub
    def normal(self, shape):
        return jax.random.normal(self._next(), shape, dtype=jnp.bfloat16)
    def randint(self, lo, hi, shape):
        return jax.random.randint(self._next(), shape, lo, hi, dtype=jnp.int32)
    def uniform(self, shape, lo=0.0, hi=1.0):
        return jax.random.uniform(self._next(), shape, jnp.bfloat16, lo, hi)
    def permutation(self, n):
        return jax.random.permutation(self._next(), n)


kernel_name = 'concat_heads__gqa_block_cached__mha_block_cached__near_ridge'

def setup_inputs():
    _rng = _Rng(jax.random.key(int.from_bytes(__import__("os").urandom(4), "little")))
    _w = (lambda a: (lambda t: t.astype(jnp.bfloat16) if jnp.issubdtype(t.dtype, jnp.floating) else t)(jnp.asarray(a)))
    def _A_setup():
        B, Sq, D = 16, 32, 512
        Hq, Hkv, Sk, Dh = 32, 8, 512, 128
        assert Hq % Hkv == 0, (Hq, Hkv)
        return {
            "x": _w((lambda *s: _rng.normal(s) * 0.8)(B, Sq, D)),
            "k_cache": _w((lambda *s: _rng.normal(s) * 0.8)(B, Hkv, Sk, Dh)),
            "v_cache": _w((lambda *s: _rng.normal(s) * 0.05)(B, Hkv, Sk, Dh)),
            "wq": _w((lambda *s: _rng.normal(s) * 0.8)(D, Hq * Dh) * (D ** -0.5)),
            "wo": _w((lambda *s: _rng.normal(s) * 0.05)(Hq * Dh, D) * ((Hq * Dh) ** -0.5)),
        }
    _A_in = _A_setup()

    def _B_setup():
        B, Sq, D = 16, 32, 512
        H, Sk, Dh = 32, 512, 128
        return {
            "x": _w((lambda *s: _rng.normal(s) * 0.8)(B, Sq, D)),
            "k_cache": _w((lambda *s: _rng.normal(s) * 0.8)(B, H, Sk, Dh)),
            "v_cache": _w((lambda *s: _rng.normal(s) * 0.05)(B, H, Sk, Dh)),
            "wq": _w((lambda *s: _rng.normal(s) * 0.8)(D, H * Dh) * (D ** -0.5)),
            "wo": _w((lambda *s: _rng.normal(s) * 0.05)(H * Dh, D) * ((H * Dh) ** -0.5)),
        }
    _B_in = _B_setup()

    return {
        "A_x": _A_in["x"],
        "A_k_cache": _A_in["k_cache"],
        "A_v_cache": _A_in["v_cache"],
        "A_wq": _A_in["wq"],
        "A_wo": _A_in["wo"],
        "B_x": _B_in["x"],
        "B_k_cache": _B_in["k_cache"],
        "B_v_cache": _B_in["v_cache"],
        "B_wq": _B_in["wq"],
        "B_wo": _B_in["wo"],
    }

def reference(A_x, A_k_cache, A_v_cache, A_wq, A_wo, B_x, B_k_cache, B_v_cache, B_wq, B_wo):
    def _A_ref(x, k_cache, v_cache, wq, wo):
        B, Sq, D = x.shape
        Hq, Dh = 32, 128
        Hkv = k_cache.shape[1]
        rep = Hq // Hkv
        q = (lambda x, *d: x.transpose(*d))((x @ wq).reshape(B, Sq, Hq, Dh), 0, 2, 1, 3)
        k = jnp.repeat(k_cache, rep, axis=1)
        v = jnp.repeat(v_cache, rep, axis=1)
        scores = jnp.einsum("bhqd,bhkd->bhqk", q, k) * (Dh ** -0.5)
        p = _softmax(scores, axis=-1)
        o = jnp.einsum("bhqk,bhkd->bhqd", p, v)
        return (lambda x, *d: x.transpose(*d))(o, 0, 2, 1, 3).reshape(B, Sq, Hq * Dh) @ wo

    def _B_ref(x, k_cache, v_cache, wq, wo):
        B, Sq, D = x.shape
        H, Dh = 32, 128
        q = (lambda x, *d: x.transpose(*d))((x @ wq).reshape(B, Sq, H, Dh), 0, 2, 1, 3)
        scores = jnp.einsum("bhqd,bhkd->bhqk", q, k_cache) * (Dh ** -0.5)
        p = _softmax(scores, axis=-1)
        o = jnp.einsum("bhqk,bhkd->bhqd", p, v_cache)
        return (lambda x, *d: x.transpose(*d))(o, 0, 2, 1, 3).reshape(B, Sq, H * Dh) @ wo

    a = _A_ref(A_x, A_k_cache, A_v_cache, A_wq, A_wo)
    b = _B_ref(B_x, B_k_cache, B_v_cache, B_wq, B_wo)
    return jnp.concatenate([a, b], axis=-1)
```

```python
import jax
import jax.numpy as jnp
from jax import lax
import jax.experimental.pallas as pl
import jax.experimental.pallas.tpu as pltpu

B, SQ, D = 16, 32, 512
H, HKV, SK, DH = 32, 8, 512, 128
REP = H // HKV
M = B * SQ
GW = REP * DH
GB = 4
RB = GB * SQ
NC = B // GB
NT = HKV * NC
NTILE = SK // 128
HEADS = ("A", 0, 1, 2, 3)
EVENTS = [(h, k, a) for h in HEADS for k in range(NTILE) for a in range(2)]
NE = len(EVENTS)
LAG = NE // len(HEADS)
AHEAD = 11
WRITE_EARLY = 4
PW, NR = 16, 4
EXP_SCALE = DH ** -0.5 * 1.4426950408889634
bf16, f32 = jnp.bfloat16, jnp.float32


def _aligned(x, n):
    return x if isinstance(x, int) else pl.multiple_of(x, n)


def _kernel(xa_h, ka_h, va_h, wqa_h, woa_h, xb_h, kb_h, vb_h, wqb_h, wob_h, out_h,
            x_v, wq_v, wo_v, kv_v, q_v, o_v, acc, stage, sems):
    def start_split(src, dst, sem):
        pltpu.make_async_copy(src.at[pl.ds(0, 1)], dst.at[pl.ds(0, 1)], sem).start(priority=0)
        pltpu.make_async_copy(src.at[pl.ds(1, 3)], dst.at[pl.ds(1, 3)], sem).start(priority=1)

    def wait_filled(dst, sem):
        pltpu.make_async_copy(dst, dst, sem).wait()

    def event_refs(t, i):
        h, k, a = EVENTS[i]
        g, c = t // NC, t % NC
        if h == "A":
            src = (ka_h, va_h)[a].at[pl.ds(c * GB, GB), g]
        else:
            src = (kb_h, vb_h)[a].at[pl.ds(c * GB, GB), g * REP + h]
        dst = kv_v.at[(t % 2) * len(HEADS) + HEADS.index(h), a]
        rows = pl.ds(k * 128, 128)
        return src.at[:, rows], dst.at[:, rows]

    def tick(t, n, last):
        if n >= NE and last:
            return
        tw, nw = (t + 1, n - NE) if n >= NE else (t, n)
        wait_filled(event_refs(tw, nw)[1], sems.at[nw])
        n += AHEAD
        if n >= NE and last:
            return
        ts, ns = (t + 1, n - NE) if n >= NE else (t, n)
        start_split(*event_refs(ts, ns), sems.at[ns])

    def q_proj(t, br):
        g, c = t // NC, t % NC
        x = x_v[br, pl.ds(_aligned(c * RB, RB), RB), :]
        w = wq_v[br, :, :, :, pl.ds(_aligned(g * GW, GW), GW)].reshape(D, GW)
        q_v[t % 2, br] = jnp.dot(x, w, preferred_element_type=f32).astype(bf16)

    def o_proj(t, br, final=False):
        g, c = t // NC, t % NC
        rows = pl.ds(_aligned(c * RB, RB), RB)
        y = jnp.dot(o_v[t % 2, br], wo_v[br, g // 2, g % 2], preferred_element_type=f32)
        y = y + acc[br, rows, :]
        if final:
            stage[rows, br * D:(br + 1) * D] = y.astype(bf16)
        else:
            acc[br, rows, :] = y

    def scores(t, h, bb):
        par, rows = t % 2, slice(bb * SQ, (bb + 1) * SQ)
        k = kv_v[par * len(HEADS) + HEADS.index(h), 0, bb]
        if h == "A":
            q = jnp.concatenate(
                [q_v[par, 0, rows, r * DH:(r + 1) * DH] for r in range(REP)], axis=0)
        else:
            q = q_v[par, 1, rows, h * DH:(h + 1) * DH]
        s = lax.dot_general(q, k, (((1,), (1,)), ((), ())), preferred_element_type=f32)
        p = jnp.exp2((s - jnp.max(s, axis=-1, keepdims=True)) * EXP_SCALE)
        l = jnp.sum(p, axis=-1, keepdims=True)
        r = pl.reciprocal(l, approx=True)
        r = r * (2.0 - l * r)
        return p.astype(bf16), r

    def values(t, h, bb, p, r):
        par, rows = t % 2, slice(bb * SQ, (bb + 1) * SQ)
        v = kv_v[par * len(HEADS) + HEADS.index(h), 1, bb]
        o = (jnp.dot(p, v, preferred_element_type=f32) * r).astype(bf16)
        if h == "A":
            for j in range(REP):
                o_v[par, 0, rows, j * DH:(j + 1) * DH] = o[j * SQ:(j + 1) * SQ]
        else:
            o_v[par, 1, rows, h * DH:(h + 1) * DH] = o

    out_copies = [
        pltpu.make_async_copy(stage.at[idx], out_h.at[idx], sems.at[NE + n])
        for n, idx in enumerate((
            (pl.ds(0, M - RB),),
            (pl.ds(M - RB, RB), pl.ds(0, D)),
            (pl.ds(M - RB, RB), pl.ds(D, D)),
        ))
    ]

    def projections(t, h, first, last):
        if not last:
            if h < 2:
                q_proj(t + 1, h)
            elif not first:
                o_proj(t - 1, h - 2)
        elif h == 0:
            o_proj(t - 1, 0, True)
            o_proj(t, 0, True)
        elif h == 1:
            o_proj(t - 1, 1, True)
            done = (NC - 2) * RB
            for br in range(2):
                stage[0:done, br * D:(br + 1) * D] = acc[br, 0:done, :].astype(bf16)
        elif h == 3:
            o_proj(t, 1, True)

    def super_step(t, first=False, last=False):
        n = LAG
        for h in HEADS:
            order = [("K", 0)]
            for bb in range(GB):
                if bb + 1 < GB:
                    order.append(("K", bb + 1))
                order.append(("V", bb))
            probs = {}
            for kind, bb in order:
                if kind == "K":
                    probs[bb] = scores(t, h, bb)
                else:
                    values(t, h, bb, *probs.pop(bb))
                tick(t, n, last)
                if last and n == NE - WRITE_EARLY:
                    for cp in out_copies[:-1]:
                        cp.start()
                n += 1
            if h != "A":
                projections(t, h, first, last)

    ps = NE + len(out_copies)

    def weight_refs(w, rnd, j):
        br, k = j % 2, (rnd % 2) * 8 + j // 2
        odd = rnd // 2
        if w == 0:
            src, dst = (wqa_h, wqb_h)[br], wq_v.at[br]
            idx = (slice(None), odd, pl.ds(_aligned((k // 2) * 8, 8), 8),
                   pl.ds((j // 2 % 2) * 2048, 2048))
        else:
            src, dst = (woa_h, wob_h)[br], wo_v.at[br]
            idx = (slice(None), odd, pl.ds(_aligned(k * 32, 32), 32))
        return src.at[idx], dst.at[idx]

    def start_weight(w, rnd, j, wrap):
        if j >= PW:
            rnd, j = (0 if wrap else rnd + 1), j - PW
            w += wrap
        if w == 2:
            start_split(*event_refs(0, j), sems.at[j])
        else:
            start_split(*weight_refs(w, rnd, j), sems.at[ps + (rnd % 2) * PW + j])

    def weight_round(w, rnd, wrap=0):
        for j in range(PW):
            wait_filled(weight_refs(w, rnd, j)[1], sems.at[ps + (rnd % 2) * PW + j])
            start_weight(w, rnd, j + AHEAD, wrap)
            if w == 0 and j % 2 == 0:
                br, rows = (j // 2) % 2, pl.ds(_aligned((rnd * 4 + j // 4) * 32, 32), 32)
                pltpu.make_async_copy((xa_h, xb_h)[br].at[rows], x_v.at[br, rows],
                                      sems.at[ps + 2 * PW]).start(priority=1)

    for j in range(AHEAD):
        start_weight(0, 0, j, 0)
    acc[...] = jnp.zeros_like(acc)
    for w in range(2):
        lax.fori_loop(0, NR - 1, lambda r, _, w=w: weight_round(w, r), None)
        weight_round(w, NR - 1, 1)
    wait_filled(x_v, sems.at[ps + 2 * PW])
    for n in range(LAG):
        tick(0, n, False)
        if n in (LAG // 4, LAG // 2):
            q_proj(0, int(n == LAG // 2))

    super_step(0, first=True)
    lax.fori_loop(1, NT - 1, lambda t, _: super_step(t), None)
    super_step(NT - 1, last=True)
    out_copies[-1].start()
    for cp in out_copies:
        cp.wait()


@jax.jit
def pallas_concat_heads__gqa_block_cached__mha_block_cached__near_ridge_kernel(
    A_x: jax.Array,
    A_k_cache: jax.Array,
    A_v_cache: jax.Array,
    A_wq: jax.Array,
    A_wo: jax.Array,
    B_x: jax.Array,
    B_k_cache: jax.Array,
    B_v_cache: jax.Array,
    B_wq: jax.Array,
    B_wo: jax.Array,
):
    wq_shape = (4, 2, D // 8, H * DH)
    wo_shape = (4, 2, H * DH // 8, D)
    out = pl.pallas_call(
        _kernel,
        in_specs=[pl.BlockSpec(memory_space=pl.ANY)] * 10,
        out_specs=pl.BlockSpec(memory_space=pl.ANY),
        out_shape=jax.ShapeDtypeStruct((M, 2 * D), bf16),
        scratch_shapes=[
            pltpu.VMEM((2, M, D), bf16),
            pltpu.VMEM((2, *wq_shape), bf16),
            pltpu.VMEM((2, *wo_shape), bf16),
            pltpu.VMEM((2 * len(HEADS), 2, GB, SK, DH), bf16),
            pltpu.VMEM((2, 2, RB, GW), bf16),
            pltpu.VMEM((2, 2, RB, GW), bf16),
            pltpu.VMEM((2, M, D), f32),
            pltpu.VMEM((M, 2 * D), bf16),
            pltpu.SemaphoreType.DMA((NE + 3 + 2 * PW + 1,)),
        ],
        compiler_params=pltpu.CompilerParams(
            vmem_limit_bytes=64 * 1024 * 1024,
            disable_bounds_checks=True,
            flags={"XLA_TPU_RESCHEDULE_DMA_DONES": True},
        ),
    )(
        A_x.reshape(M, D), A_k_cache, A_v_cache, A_wq.reshape(wq_shape), A_wo.reshape(wo_shape),
        B_x.reshape(M, D), B_k_cache, B_v_cache, B_wq.reshape(wq_shape), B_wo.reshape(wo_shape),
    )
    return out.reshape(B, SQ, 2 * D)
```

```python
import jax
import jax.numpy as jnp
from jax import lax
import jax.experimental.pallas as pl
import jax.experimental.pallas.tpu as pltpu

B, SQ, D = 16, 32, 512
H, HKV, SK, DH = 32, 8, 512, 128
REP = H // HKV
GW = REP * DH
GB = 4
NC = B // GB
RB = GB * SQ
NT = HKV * NC
TILE = 128
NTILE = SK // TILE
EXP_SCALE = DH ** -0.5 * 1.4426950408889634

AHEAD = (8, 12)
WRITE_EARLY = 5
NSEM = 32
W_AHEAD, W_ROUND, W_ROUNDS = 10, 16, 4

bf16, f32 = jnp.bfloat16, jnp.float32


def _events():
    def mha(j):
        return [("B", j, a, b, 2, k * TILE, TILE)
                for k in range(NTILE) for a in range(2) for b in (0, 2)]

    def mha_only(j, a, k):
        return ("B", j, a, 0, 1, k * TILE, TILE), ("B", j, a, 1, GB - 1, k * TILE, TILE)

    usual = []
    for j in range(REP):
        gqa = [("A", j, a, r + u, TILE // 2)
               for r in range(0, SK, TILE) for a in range(2) for u in (0, TILE // 2)]
        usual.append(list(zip(gqa, mha(j))))
    last = []
    for j in range(2):
        gqa = [("A", 2 * j + d, a, r, TILE)
               for r in range(0, SK, TILE) for a in range(2) for d in range(2)]
        last.append(list(zip(gqa, mha(j))))
    for a in range(2):
        last.append([mha_only(j, a, k) for k in range(NTILE) for j in (2, 3)])
    return usual, last


STEPS, STEPS_LAST = _events()
EVENTS = [e for s in STEPS for e in s]
EVENTS_LAST = [e for s in STEPS_LAST for e in s]
NE = len(EVENTS)
OUT_EARLY = [(slice(None), pl.ds(0, NC - 1))] + [
    (i, NC - 1, slice(None), pl.ds(0, D)) for i in range(GB)]
OUT_LATE = [(i, NC - 1, slice(None), pl.ds(D, D)) for i in range(GB)]
SEM_GQA = NSEM
SEM_OUT = SEM_GQA + 2 * GB * 2
SEM_W = SEM_OUT + len(OUT_EARLY) + len(OUT_LATE)
SEM_X = SEM_W + 2 * W_ROUND


def _aligned(x, n):
    return x if isinstance(x, int) else pl.multiple_of(x, n)


def _kernel(xa_h, ka_h, va_h, wqa_h, woa_h, xb_h, kb_h, vb_h, wqb_h, wob_h, out_h,
            x_v, wq_v, wo_v, kv_v, q_v, o_v, acc, stage, sems):

    def wait_filled(dst, sem):
        pltpu.make_async_copy(dst, dst, sem).wait()

    def gqa_sem(t, b, a):
        return sems.at[SEM_GQA + (t % 2) * GB * 2 + b * 2 + a]

    def piece_refs(t, piece):
        g, c = t // NC, t % NC
        slot = (t % 2) * (1 + REP)
        if piece[0] == "B":
            _, j, a, b, nb, r, n = piece
            bs, rows = pl.ds(b, nb), pl.ds(r, n)
            return (kb_h, vb_h)[a].at[bs, c, g * REP + j, rows], kv_v.at[slot + 1 + j, a, bs, rows]
        _, b, a, r, n = piece
        rows = pl.ds(r, n)
        return (ka_h, va_h)[a].at[b, c, g, rows], kv_v.at[slot, a, b, rows]

    def start_piece(t, n, events, queue):
        piece = events[n][queue]
        sem = sems.at[n % NSEM] if piece[0] == "B" else gqa_sem(t, piece[1], piece[2])
        pltpu.make_async_copy(*piece_refs(t, piece), sem).start(priority=queue)

    def tick(t, n, last):
        events = EVENTS_LAST if last else EVENTS
        tw, nw = (t, n) if n < NE else (t + 1, n - NE)
        q0, q1 = events[nw]
        assert n < NE or q1 == EVENTS_LAST[nw][1]
        filled = q0[:4] + (GB,) + q0[5:] if q0[0] == "B" else q1
        wait_filled(piece_refs(tw, filled)[1], sems.at[nw % NSEM])
        for queue in range(2):
            m = n + AHEAD[queue]
            if m < len(events):
                start_piece(t, m, events, queue)
            elif last:
                pass
            elif EVENTS[m - NE][queue] == EVENTS_LAST[m - NE][queue]:
                start_piece(t + 1, m - NE, EVENTS, queue)
            else:
                pl.when(t < NT - 2)(lambda: start_piece(t + 1, m - NE, EVENTS, queue))
                pl.when(t == NT - 2)(lambda: start_piece(t + 1, m - NE, EVENTS_LAST, queue))

    def q_proj(t, br, c0, c1):
        g, c = t // NC, t % NC
        x = x_v[br, :, c].reshape(RB, D)
        cols = pl.ds(_aligned(g * GW + c0, DH), c1 - c0)
        w = wq_v[br, :, :, :, cols].reshape(D, c1 - c0)
        q_v[t % 2, br, :, c0:c1] = jnp.dot(x, w, preferred_element_type=f32).astype(bf16)

    def to_stage(c, br, y):
        stage[:, c, :, br * D:(br + 1) * D] = y.astype(bf16).reshape(GB, SQ, D)

    def o_proj(t, br, final=False, k0=0, k1=GW, c0=0, c1=D):
        g, c = t // NC, t % NC
        w = wo_v[br, g // 2, g % 2, k0:k1, c0:c1]
        y = jnp.dot(o_v[t % 2, br, :, k0:k1], w, preferred_element_type=f32)
        y = y + acc[br, c, :, c0:c1]
        if final:
            to_stage(c, br, y)
        else:
            acc[br, c, :, c0:c1] = y

    def scores(t, h, b):
        par, rows = t % 2, slice(b * SQ, (b + 1) * SQ)
        if h == "A":
            q = jnp.concatenate(
                [q_v[par, 0, rows, r * DH:(r + 1) * DH] for r in range(REP)], axis=0)
        else:
            q = q_v[par, 1, rows, h * DH:(h + 1) * DH]
        k = kv_v[par * (1 + REP) + (0 if h == "A" else 1 + h), 0, b]
        s = lax.dot_general(q, k, (((1,), (1,)), ((), ())), preferred_element_type=f32)
        p = jnp.exp2((s - jnp.max(s, axis=-1, keepdims=True)) * EXP_SCALE)
        return p.astype(bf16), 1.0 / jnp.sum(p, axis=-1, keepdims=True)

    def values(t, h, b, p, inv_sum):
        par, rows = t % 2, slice(b * SQ, (b + 1) * SQ)
        v = kv_v[par * (1 + REP) + (0 if h == "A" else 1 + h), 1, b]
        o = (jnp.dot(p, v, preferred_element_type=f32) * inv_sum).astype(bf16)
        if h == "A":
            for r in range(REP):
                o_v[par, 0, rows, r * DH:(r + 1) * DH] = o[r * SQ:(r + 1) * SQ]
        else:
            o_v[par, 1, rows, h * DH:(h + 1) * DH] = o

    out_copies = [
        pltpu.make_async_copy(stage.at[idx], out_h.at[idx], sems.at[SEM_OUT + n])
        for n, idx in enumerate(OUT_EARLY + OUT_LATE)]

    def step_tasks(j, last):
        if last and j >= 2:
            return [("KV"[j - 2], h, b) for h in (2, 3) for b in range(GB)]
        items = [(j, b) for b in range(GB)]
        items[2:2] = [("A", 2 * j), ("A", 2 * j + 1)] if last else [("A", j)]
        tasks = [("K",) + items[0]]
        for i, item in enumerate(items):
            if i + 1 < len(items):
                tasks.append(("K",) + items[i + 1])
            tasks.append(("V",) + item)
        if not last:
            for u in reversed(range(REP)):
                tasks.insert(2 * u + 2, ("P", u * DH, (u + 1) * DH))
        return tasks

    def super_step(t, last):
        steps = STEPS_LAST if last else STEPS + STEPS[:1]
        n = len(steps[0])
        probs = {}
        for j in range(REP):
            tasks = step_tasks(j, last)
            first, todo = n, len(steps[j + 1]) if j + 1 < len(steps) else 0
            for i, (kind, u, v) in enumerate(tasks):
                if kind == "K":
                    if u == "A":
                        for a in range(2):
                            wait_filled(piece_refs(t, ("A", v, a, 0, SK))[1], gqa_sem(t, v, a))
                    probs[u, v] = scores(t, u, v)
                elif kind == "V":
                    values(t, u, v, *probs.pop((u, v)))
                elif j < 2:
                    q_proj(t + 1, j, u, v)
                else:
                    o_proj(jnp.where(t > 0, t - 1, NC - 1), j - 2, c0=u, c1=v)
                if last and (kind, u, v) == ("V", 2, GB - 1):
                    o_proj(t, 1, k1=3 * DH)
                while n < first + pl.cdiv(todo * (i + 1), len(tasks)):
                    tick(t, n, last)
                    if last and n == len(EVENTS_LAST) - WRITE_EARLY:
                        assert j >= 2
                        for cp in out_copies[:len(OUT_EARLY)]:
                            cp.start()
                    n += 1
            if last and j == 0:
                o_proj(t - 1, 0, final=True)
                o_proj(t - 1, 1, final=True)
            if last and j == 1:
                for br in range(2):
                    for c in range(NC - 2):
                        to_stage(c, br, acc[br, c])
                o_proj(t, 0, final=True)
            if last and j == 3:
                o_proj(t, 1, final=True, k0=3 * DH)

    def weight_refs(w, rnd, j):
        br, k, odd = j % 2, (rnd % 2) * 8 + j // 2, rnd // 2
        if w == 0:
            src, dst = (wqa_h, wqb_h)[br], wq_v.at[br]
            idx = (slice(None), odd, pl.ds(_aligned((k // 2) * 8, 8), 8),
                   pl.ds((j // 2 % 2) * 2048, 2048))
        else:
            src, dst = (woa_h, wob_h)[br], wo_v.at[br]
            idx = (slice(None), odd, pl.ds(_aligned(k * 32, 32), 32))
        return src.at[idx], dst.at[idx]

    def start_weight(w, rnd, j, wrap):
        if j >= W_ROUND:
            rnd, j = (0 if wrap else rnd + 1), j - W_ROUND
            w += wrap
        if w == 2:
            for n in range(j * max(AHEAD) // W_AHEAD, (j + 1) * max(AHEAD) // W_AHEAD):
                for queue in range(2):
                    if n < AHEAD[queue]:
                        start_piece(0, n, EVENTS, queue)
            return
        src, dst = weight_refs(w, rnd, j)
        sem = sems.at[SEM_W + (rnd % 2) * W_ROUND + j]
        for queue, part in enumerate((pl.ds(0, 1), pl.ds(1, 3))):
            pltpu.make_async_copy(src.at[part], dst.at[part], sem).start(priority=queue)

    def weight_round(w, rnd, wrap=0):
        for j in range(W_ROUND):
            wait_filled(weight_refs(w, rnd, j)[1], sems.at[SEM_W + (rnd % 2) * W_ROUND + j])
            start_weight(w, rnd, j + W_AHEAD, wrap)
            if w == 0 and j % 2 == 0:
                br, idx = (j // 2) % 2, (rnd, j // 4)
                pltpu.make_async_copy((xa_h, xb_h)[br].at[idx], x_v.at[(br,) + idx],
                                      sems.at[SEM_X]).start(priority=1)

    for j in range(W_AHEAD):
        start_weight(0, 0, j, 0)
    acc[...] = jnp.zeros_like(acc)
    o_v[1] = jnp.zeros(o_v.shape[1:], bf16)
    for w in range(2):
        lax.fori_loop(0, W_ROUNDS - 1, lambda r, _, w=w: weight_round(w, r), None)
        weight_round(w, W_ROUNDS - 1, 1)
    wait_filled(x_v, sems.at[SEM_X])
    for n in range(len(STEPS[0])):
        tick(0, n, False)
        if n % 2 == 1:
            u = n // 2
            q_proj(0, u // REP, (u % REP) * DH, (u % REP + 1) * DH)

    lax.fori_loop(0, NT - 1, lambda t, _: super_step(t, False), None)
    super_step(NT - 1, True)
    for cp in out_copies[len(OUT_EARLY):]:
        cp.start()
    for cp in out_copies:
        cp.wait()


@jax.jit
def pallas_concat_heads__gqa_block_cached__mha_block_cached__near_ridge_kernel(
    A_x: jax.Array,
    A_k_cache: jax.Array,
    A_v_cache: jax.Array,
    A_wq: jax.Array,
    A_wo: jax.Array,
    B_x: jax.Array,
    B_k_cache: jax.Array,
    B_v_cache: jax.Array,
    B_wq: jax.Array,
    B_wo: jax.Array,
):
    def by_chunk(a):
        return a.reshape(GB, NC, *a.shape[1:])

    wq_shape = (4, 2, D // 8, H * DH)
    wo_shape = (4, 2, H * DH // 8, D)
    out = pl.pallas_call(
        _kernel,
        in_specs=[pl.BlockSpec(memory_space=pl.ANY)] * 10,
        out_specs=pl.BlockSpec(memory_space=pl.ANY),
        out_shape=jax.ShapeDtypeStruct((GB, NC, SQ, 2 * D), bf16),
        scratch_shapes=[
            pltpu.VMEM((2, GB, NC, SQ, D), bf16),
            pltpu.VMEM((2, *wq_shape), bf16),
            pltpu.VMEM((2, *wo_shape), bf16),
            pltpu.VMEM((2 * (1 + REP), 2, GB, SK, DH), bf16),
            pltpu.VMEM((2, 2, RB, GW), bf16),
            pltpu.VMEM((2, 2, RB, GW), bf16),
            pltpu.VMEM((2, NC, RB, D), f32),
            pltpu.VMEM((GB, NC, SQ, 2 * D), bf16),
            pltpu.SemaphoreType.DMA((SEM_X + 1,)),
        ],
        compiler_params=pltpu.CompilerParams(
            vmem_limit_bytes=64 * 1024 * 1024,
            disable_semaphore_checks=True,
            flags={"XLA_TPU_RESCHEDULE_DMA_DONES": True},
        ),
    )(
        by_chunk(A_x), by_chunk(A_k_cache), by_chunk(A_v_cache),
        A_wq.reshape(wq_shape), A_wo.reshape(wo_shape),
        by_chunk(B_x), by_chunk(B_k_cache), by_chunk(B_v_cache),
        B_wq.reshape(wq_shape), B_wo.reshape(wo_shape),
    )
    return out.reshape(B, SQ, 2 * D)
```
